```python
import jax
import jax.numpy as jnp

def _softmax(x, axis=-1):
    return jax.nn.softmax(x, axis=axis)
def _gelu(x):
    return jax.nn.gelu(x, approximate=True)
def _silu(x):
    return jax.nn.silu(x)
def _sigmoid(x):
    return jax.nn.sigmoid(x)
def _layernorm(x, axis=-1, eps=1e-5):
    m = jnp.mean(x, axis=axis, keepdims=True)
    v = jnp.var(x, axis=axis, keepdims=True)
    return (x - m) / jnp.sqrt(v + eps)
def _scatter_add(tgt, idx, src, axis=0):
    return tgt.at[idx].add(src)
def _segment_sum(src, seg, n):
    return jax.ops.segment_sum(src, seg, n)
class _Rng:
    def __init__(self, key):
        self._k = key
    def _next(self):
        self._k, sub = jax.random.split(self._k)
        return sub
    def normal(self, shape):
        return jax.random.normal(self._next(), shape, dtype=jnp.bfloat16)
    def randint(self, lo, hi, shape):
        return jax.random.randint(self._next(), shape, lo, hi, dtype=jnp.int32)
    def uniform(self, shape, lo=0.0, hi=1.0):
        return jax.random.uniform(self._next(), shape, jnp.bfloat16, lo, hi)
    def permutation(self, n):
        return jax.random.permutation(self._next(), n)


kernel_name = 'interleave_layers__sliding_block_cached__dense_activation_gelu__decode'

def _fwd_setup_inputs():
    _rng = _Rng(jax.random.key(int.from_bytes(__import__("os").urandom(4), "little")))
    _w = (lambda a: (lambda t: t.astype(jnp.bfloat16) if jnp.issubdtype(t.dtype, jnp.floating) else t)(jnp.asarray(a)))
    def _A_setup():
        B, Sq, D = 2, 1, 512
        Hq, Hkv, Sk, Dh = 32, 8, 32768, 128
        assert Hq % Hkv == 0, (Hq, Hkv)
        return {
            "x": _w((lambda *s: _rng.normal(s) * 0.05)(B, Sq, D)),
            "k_cache": _w((lambda *s: _rng.normal(s) * 0.05)(B, Hkv, Sk, Dh)),
            "v_cache": _w((lambda *s: _rng.normal(s) * 0.05)(B, Hkv, Sk, Dh)),
            "wq": _w((lambda *s: _rng.normal(s) * 0.05)(D, Hq * Dh) * (D ** -0.5)),
            "wo": _w((lambda *s: _rng.normal(s) * 0.05)(Hq * Dh, D) * ((Hq * Dh) ** -0.5)),
        }
    _A_in = _A_setup()

    def _B_setup():
        B, S, D, F = 2, 1, 512, 1792
        return {
            "x": _w((lambda *s: _rng.normal(s) * 0.05)(B, S, D)),
            "w1": _w((lambda *s: _rng.normal(s) * 0.05)(D, F) * (D ** -0.5)),
            "b1": _w((lambda *s: _rng.normal(s) * 0.05)(F) * 0.01),
            "w2": _w((lambda *s: _rng.normal(s) * 0.05)(F, D) * (F ** -0.5)),
            "b2": _w((lambda *s: _rng.normal(s) * 0.05)(D) * 0.01),
        }
    _B_in = _B_setup()

    return {
        "A_x": _A_in["x"],
        "A_k_cache": _A_in["k_cache"],
        "A_v_cache": _A_in["v_cache"],
        "A_wq": _A_in["wq"],
        "A_wo": _A_in["wo"],
        "B_x": _B_in["x"],
        "B_w1": _B_in["w1"],
        "B_b1": _B_in["b1"],
        "B_w2": _B_in["w2"],
        "B_b2": _B_in["b2"],
    }

def _fwd_reference(A_x, A_k_cache, A_v_cache, A_wq, A_wo, B_x, B_w1, B_b1, B_w2, B_b2):
    def _A_ref(x, k_cache, v_cache, wq, wo):
        B, Sq, D = x.shape
        Hq, Dh = 32, 128
        Hkv, Sk = k_cache.shape[1], k_cache.shape[2]
        W = min(4096, max(256, Sk // 4))
        rep = Hq // Hkv
        q = (lambda x, *d: x.transpose(*d))((x @ wq).reshape(B, Sq, Hq, Dh), 0, 2, 1, 3)
        k = jnp.repeat(k_cache[:, :, Sk - W:, :], rep, axis=1)
        v = jnp.repeat(v_cache[:, :, Sk - W:, :], rep, axis=1)
        scores = jnp.einsum("bhqd,bhkd->bhqk", q, k) * (Dh ** -0.5)
        p = _softmax(scores, axis=-1)
        o = jnp.einsum("bhqk,bhkd->bhqd", p, v)
        return (lambda x, *d: x.transpose(*d))(o, 0, 2, 1, 3).reshape(B, Sq, Hq * Dh) @ wo

    def _B_ref(x, w1, b1, w2, b2):
        h = jnp.einsum("bsd,df->bsf", x, w1) + b1
        h = _gelu(h)
        return jnp.einsum("bsf,fd->bsd", h, w2) + b2

    x = A_x
    x = x + _A_ref(_layernorm(x, axis=-1), A_k_cache, A_v_cache, A_wq, A_wo)
    x = x + _B_ref(_layernorm(x, axis=-1), B_w1, B_b1, B_w2, B_b2)
    x = x + _A_ref(_layernorm(x, axis=-1), A_k_cache, A_v_cache, A_wq, A_wo)
    x = x + _B_ref(_layernorm(x, axis=-1), B_w1, B_b1, B_w2, B_b2)
    return x


def setup_inputs():
    _inp = _fwd_setup_inputs()
    _gk = jax.random.fold_in(jax.random.key(int.from_bytes(__import__("os").urandom(4), "little")), 2**31 - 1)
    _shapes = [[2, 1, 512]]
    _dtypes = ['bfloat16']
    _gks = jax.random.split(_gk, len(_shapes))
    _gs = [jax.random.normal(k, s, dtype=jnp.dtype(d)) * 0.05 for k, s, d in zip(_gks, _shapes, _dtypes)]
    _inp["grad_out"] = _gs[0]
    return _inp

def reference(A_x, A_k_cache, A_v_cache, A_wq, A_wo, B_w1, B_b1, B_w2, B_b2, B_x, grad_out):
    _const = dict(B_x=B_x)
    def _f(*_d):
        return _fwd_reference(**{'A_x': _d[0], 'A_k_cache': _d[1], 'A_v_cache': _d[2], 'A_wq': _d[3], 'A_wo': _d[4], 'B_w1': _d[5], 'B_b1': _d[6], 'B_w2': _d[7], 'B_b2': _d[8], **_const})
    _out, _vjp = jax.vjp(_f, A_x, A_k_cache, A_v_cache, A_wq, A_wo, B_w1, B_b1, B_w2, B_b2)
    _grads = _vjp(grad_out)
    _out0 = jnp.asarray(_out)
    return (_out0, *[jnp.asarray(_g) for _g in _grads])
```

```python
import math

import jax
import jax.numpy as jnp
from jax import lax
import jax.experimental.pallas as pl
import jax.experimental.pallas.tpu as pltpu

F32 = jnp.float32
BF16 = jnp.bfloat16

HQ = 32
LN_EPS = 1e-5
ROWS = 8

_NN = (((1,), (0,)), ((), ()))
_NT = (((1,), (1,)), ((), ()))
_TN = (((0,), (0,)), ((), ()))

_GELU_C = math.sqrt(2.0 / math.pi)
_GELU_A = 0.044715

RSEG, RROWS = 4, 32
WSEG, WROWS = 4, 64
PIECES = ((16, 1024), (32, 512), (64, 256), (32, 512))


def _mm(a, b, dims):
    return lax.dot_general(a.astype(BF16), b, dims, preferred_element_type=F32)


def _ln_fwd(x):
    xc = x - jnp.mean(x, axis=-1, keepdims=True)
    rstd = 1.0 / jnp.sqrt(jnp.mean(xc * xc, axis=-1, keepdims=True) + LN_EPS)
    return xc * rstd, rstd


def _ln_bwd(dh, h, rstd):
    return rstd * (dh - jnp.mean(dh, axis=-1, keepdims=True)
                   - h * jnp.mean(dh * h, axis=-1, keepdims=True))


def _gelu_fwd(a):
    t = jnp.tanh(_GELU_C * (a + _GELU_A * a * a * a))
    g = 0.5 * a * (1.0 + t)
    dg = 0.5 * (1.0 + t) + 0.5 * a * (1.0 - t * t) * (_GELU_C * (1.0 + 3.0 * _GELU_A * a * a))
    return g, dg


def _pad_rows(x):
    return jnp.concatenate([x, jnp.zeros((ROWS - x.shape[0], x.shape[1]), x.dtype)], axis=0)


def _loop(lo, hi, fn):
    if hi > lo:
        lax.fori_loop(lo, hi, lambda j, c: (fn(j), c)[1], 0)


def _num_pieces(ref, piece):
    assert ref.shape[0] % piece[0] == 0 and ref.shape[1] % piece[1] == 0
    return (ref.shape[0] // piece[0]) * (ref.shape[1] // piece[1])


def _copy_piece(src, dst, sem, piece, i, priority):
    rows, cols = piece
    nc = src.shape[1] // cols
    sl = (pl.ds(pl.multiple_of((i // nc) * rows, rows), rows),
          pl.ds(pl.multiple_of((i % nc) * cols, cols), cols))
    pltpu.make_async_copy(src.at[sl], dst.at[sl], sem).start(priority=priority)


def _interleave_weights(lo, hi, main, srcs, dsts, sems):
    for a in (0, 2):
        n = _num_pieces(srcs[a], PIECES[a])
        assert n == _num_pieces(srcs[a + 1], PIECES[a + 1])
        m = min(n, hi - lo)

        def pieces(i, a=a):
            for q in range(2):
                _copy_piece(srcs[a + q], dsts[a + q], sems[a + q], PIECES[a + q], i, q)

        _loop(0, m, lambda i, lo=lo: (main(lo + i), pieces(i)))
        _loop(m, n, pieces)
        lo += m
    _loop(lo, hi, main)


def _kernel(
    x_hbm, k_hbm, v_hbm, wq_hbm, wo_hbm, w1_hbm, b1_hbm, w2_hbm, b2_hbm, g_hbm,
    out_hbm, dx_hbm, dk_hbm, dv_hbm, dwq_hbm, dwo_hbm, dw1_hbm, db1_hbm, dw2_hbm, db2_hbm,
    kb, vb, wq, wo, w1, w2, x_s, g_s, b1_s, b2_s,
    dwq, dwo, dw1, dw2, out_s, dx_s, db1_s, db2_s,
    zero, q_t, o_t, do_t, dq_t, p_all, flat,
    ha_st, dq_st, oa_st, dxa_st, hb_st, da_st, gb_st, dxb_st,
    rsem, wsem,
):
    B, HKV, SK, DH = k_hbm.shape
    W = kb.shape[1]
    NG = B * HKV
    REP = HQ // HKV
    ZR = SK - W
    scale = DH ** -0.5

    def strip(j, seg, rows, extent):
        per = extent // rows
        grp = j // per
        return grp // (HKV // seg), (grp % (HKV // seg)) * seg, (j % per) * rows

    def window_views(j, seg, rows):
        b, h, r = strip(j, seg, rows, W)
        return ((b, pl.ds(h, seg), pl.ds(pl.multiple_of(ZR + r, rows), rows)),
                (pl.ds(b * HKV + h, seg), pl.ds(pl.multiple_of(r, rows), rows)))

    def kv_read(j):
        far, near = window_views(j, RSEG, RROWS)
        for i, (src, dst) in enumerate(((k_hbm, kb), (v_hbm, vb))):
            pltpu.make_async_copy(src.at[far], dst.at[near], rsem.at[i]).start(priority=i)

    n_read = (NG // RSEG) * (W // RROWS)
    head_start = min(16, n_read)
    _loop(0, head_start, kv_read)
    for i, (src, dst) in enumerate(((x_hbm, x_s), (g_hbm, g_s), (b1_hbm, b1_s), (b2_hbm, b2_s))):
        pltpu.make_async_copy(src, dst, rsem.at[6 + i]).start()
    for ref in (zero, q_t, do_t, flat, ha_st, dq_st, oa_st, dxa_st, hb_st, da_st, gb_st, dxb_st):
        ref[...] = jnp.zeros(ref.shape, ref.dtype)
    _interleave_weights(head_start, n_read, kv_read, (wq_hbm, wo_hbm, w1_hbm, w2_hbm),
                        (wq, wo, w1, w2), [rsem.at[2 + i] for i in range(4)])

    def zero_write(j):
        b, h, r = strip(j, WSEG, WROWS, ZR)
        for i, dst in enumerate((dk_hbm, dv_hbm)):
            pltpu.make_async_copy(
                zero, dst.at[b, pl.ds(h, WSEG), pl.ds(pl.multiple_of(r, WROWS), WROWS)],
                wsem.at[i]).start(priority=i)

    n_zero = (NG // WSEG) * (ZR // WROWS)
    n_feed = max(0, n_zero - _num_pieces(wq, PIECES[0]) - _num_pieces(w1, PIECES[2]))
    issued = [0]

    def feed(n):
        base = issued[0]
        issued[0] = min(base + n, n_feed)
        _loop(base, issued[0], zero_write)

    def head_loop(body, per_head):
        base = issued[0]
        per_head = min(per_head, (n_feed - base) // NG)
        issued[0] = base + per_head * NG

        def step(g):
            _loop(0, per_head, lambda u: zero_write(base + g * per_head + u))
            body(g)
        _loop(0, NG, step)

    feed(40)
    for i, buf in enumerate((kb, vb, wq, wo, w1, w2, x_s, g_s, b1_s, b2_s)):
        pltpu.make_async_copy(buf, buf, rsem.at[i]).wait()

    def to_tiles(val, tiles, layer):
        for b in range(B):
            for hq in range(HQ):
                row = layer * REP + hq % REP
                tiles[b * HKV + hq // REP, row:row + 1, :] = val[b:b + 1, hq * DH:(hq + 1) * DH]

    def from_tiles(tiles, layer):
        for b in range(B):
            for hq in range(HQ):
                row = layer * REP + hq % REP
                flat[b:b + 1, hq * DH:(hq + 1) * DH] = tiles[b * HKV + hq // REP, row:row + 1, :]
        return flat[...]

    def stack(ref, val, layer):
        ref[layer * B:(layer + 1) * B, :] = val[0:B, :]

    def attn_fwd(x, layer):
        h, rstd = _ln_fwd(x)
        stack(ha_st, h, layer)
        to_tiles(_mm(h, wq[...], _NN), q_t, layer)

        def body(g):
            s = _mm(q_t[g], kb[g], _NT) * scale
            e = jnp.exp(s - jnp.max(s, axis=-1, keepdims=True))
            p = e / jnp.sum(e, axis=-1, keepdims=True)
            if layer == 1:
                p_all[g] = p
            o_t[g] = _mm(p, vb[g], _NN)
        head_loop(body, 16)
        o = from_tiles(o_t, layer)
        stack(oa_st, o, layer)
        feed(16)
        return x + _mm(o, wo[...], _NN), (h, rstd)

    b1 = b1_s[...].astype(F32).reshape(1, -1)
    b2 = b2_s[...].astype(F32).reshape(1, -1)

    def mlp_fwd(x, layer):
        h, rstd = _ln_fwd(x)
        stack(hb_st, h, layer)
        g, dgelu = _gelu_fwd(_mm(h, w1[...], _NN) + b1)
        stack(gb_st, g, layer)
        feed(16)
        return x + _mm(g, w2[...], _NN) + b2, (h, rstd, dgelu)

    x0 = _pad_rows(x_s[...].astype(F32))
    x1, res_a0 = attn_fwd(x0, 0)
    x2, res_b0 = mlp_fwd(x1, 0)
    x3, res_a1 = attn_fwd(x2, 1)
    x4, res_b1 = mlp_fwd(x3, 1)
    out_s[...] = x4[0:B].astype(BF16)
    pltpu.make_async_copy(out_s, out_hbm, wsem.at[6]).start()

    def mlp_bwd(dy, res, layer):
        h, rstd, dgelu = res
        stack(dxb_st, dy, layer)
        da = _mm(dy, w2[...], _NT) * dgelu
        stack(da_st, da, layer)
        feed(16)
        return dy + _ln_bwd(_mm(da, w1[...], _NT), h, rstd)

    def attn_bwd(dy, res, layer):
        h, rstd = res
        to_tiles(_mm(dy, wo[...], _NT), do_t, layer)

        def body(g):
            p = p_all[g]
            do = do_t[g]
            dp = _mm(do, vb[g], _NT)
            ds = p * (dp - jnp.sum(p * dp, axis=-1, keepdims=True)) * scale
            dq_t[g] = _mm(ds, kb[g], _NN)
            if layer == 0:
                kb[g] = _mm(ds, q_t[g].astype(BF16), _TN).astype(BF16)
                vb[g] = _mm(p, do.astype(BF16), _TN).astype(BF16)
        head_loop(body, 16 if layer else 24)
        dq = from_tiles(dq_t, layer)
        stack(dq_st, dq, layer)
        feed(16)
        return dy + _ln_bwd(_mm(dq, wq[...], _NT), h, rstd)

    def wgrad(dst, lhs_st, rhs_st, rows):
        rhs = rhs_st[...].astype(BF16)
        for r in range(0, dst.shape[0], rows):
            dst[r:r + rows, :] = _mm(lhs_st[:, r:r + rows], rhs, _TN).astype(BF16)
        feed(16)

    d4 = _pad_rows(g_s[...].astype(F32))
    d3 = mlp_bwd(d4, res_b1, 1)
    stack(dxa_st, d3, 1)
    d2 = attn_bwd(d3, res_a1, 1)
    d1 = mlp_bwd(d2, res_b0, 0)
    stack(dxa_st, d1, 0)
    db1_s[...] = jnp.sum(da_st[...], axis=0).astype(BF16)
    db2_s[...] = jnp.sum(dxb_st[...], axis=0).astype(BF16)
    pltpu.make_async_copy(db1_s, db1_hbm, wsem.at[7]).start()
    pltpu.make_async_copy(db2_s, db2_hbm, wsem.at[8]).start()
    wgrad(dw2, gb_st, dxb_st, 256)
    wgrad(dw1, hb_st, da_st, 128)
    wgrad(dwo, oa_st, dxa_st, 512)
    d0 = attn_bwd(d1, res_a0, 0)
    dx_s[...] = d0[0:B].astype(BF16)
    pltpu.make_async_copy(dx_s, dx_hbm, wsem.at[9]).start()
    wgrad(dwq, ha_st, dq_st, 128)

    def kv_write(j):
        far, near = window_views(j, WSEG, WROWS)
        for i, (src, dst) in enumerate(((kb, dk_hbm), (vb, dv_hbm))):
            pltpu.make_async_copy(src.at[near], dst.at[far], wsem.at[i]).start(priority=i)

    feed(n_zero)
    _interleave_weights(n_feed, n_zero, zero_write, (dwq, dwo, dw1, dw2),
                        (dwq_hbm, dwo_hbm, dw1_hbm, dw2_hbm), [wsem.at[2 + i] for i in range(4)])
    _loop(0, (NG // WSEG) * (W // WROWS), kv_write)
    for i, buf in enumerate((dk_hbm, dv_hbm, dwq_hbm, dwo_hbm, dw1_hbm, dw2_hbm,
                             out_hbm, db1_hbm, db2_hbm, dx_hbm)):
        pltpu.make_async_copy(buf, buf, wsem.at[i]).wait()


@jax.jit
def pallas_interleave_layers__sliding_block_cached__dense_activation_gelu__decode_kernel(
    A_x: jax.Array,
    A_k_cache: jax.Array,
    A_v_cache: jax.Array,
    A_wq: jax.Array,
    A_wo: jax.Array,
    B_x: jax.Array,
    B_w1: jax.Array,
    B_b1: jax.Array,
    B_w2: jax.Array,
    B_b2: jax.Array,
    grad_out: jax.Array,
):
    del B_x
    B, SQ, D = A_x.shape
    _, HKV, SK, DH = A_k_cache.shape
    FF = B_w1.shape[1]
    W = min(4096, max(256, SK // 4))
    NG = B * HKV
    assert SQ == 1 and 2 * B <= ROWS and 2 * (HQ // HKV) == ROWS
    assert HKV % RSEG == 0 and HKV % WSEG == 0
    assert W % RROWS == 0 and W % WROWS == 0 and SK % RROWS == 0 and SK % WROWS == 0

    def like(a):
        return jax.ShapeDtypeStruct(a.shape, a.dtype)

    def vmem(shape, dtype=BF16):
        return pltpu.VMEM(tuple(shape), dtype)

    act = jax.ShapeDtypeStruct((B, D), A_x.dtype)
    hbm = pl.BlockSpec(memory_space=pltpu.HBM)
    weights = [vmem(w.shape) for w in (A_wq, A_wo, B_w1, B_w2)]
    small = [vmem((B, D)), vmem((B, D)), vmem((FF,)), vmem((D,))]
    tile = vmem((NG, ROWS, DH), F32)
    res = pl.pallas_call(
        _kernel,
        out_shape=(act, act, like(A_k_cache), like(A_v_cache), like(A_wq), like(A_wo),
                   like(B_w1), like(B_b1), like(B_w2), like(B_b2)),
        in_specs=[hbm] * 10,
        out_specs=(hbm,) * 10,
        scratch_shapes=[
            vmem((NG, W, DH)), vmem((NG, W, DH)), *weights, *small,
            *weights, *small,
            vmem((WSEG, WROWS, DH)), tile, tile, tile, tile,
            vmem((NG, ROWS, W), F32), vmem((ROWS, HQ * DH), F32),
            vmem((ROWS, D), F32), vmem((ROWS, HQ * DH), F32),
            vmem((ROWS, HQ * DH), F32), vmem((ROWS, D), F32),
            vmem((ROWS, D), F32), vmem((ROWS, FF), F32),
            vmem((ROWS, FF), F32), vmem((ROWS, D), F32),
            pltpu.SemaphoreType.DMA((10,)), pltpu.SemaphoreType.DMA((10,)),
        ],
        compiler_params=pltpu.CompilerParams(vmem_limit_bytes=100 * 2**20),
    )(A_x.reshape(B, D), A_k_cache, A_v_cache, A_wq, A_wo, B_w1, B_b1, B_w2, B_b2,
      grad_out.reshape(B, D))
    return (res[0].reshape(B, SQ, D), res[1].reshape(B, SQ, D), *res[2:])
```

```python
import math

import jax
import jax.numpy as jnp
from jax import lax
import jax.experimental.pallas as pl
import jax.experimental.pallas.tpu as pltpu

F32 = jnp.float32
BF16 = jnp.bfloat16

HQ = 32
LN_EPS = 1e-5
ROWS = 8

_NN = (((1,), (0,)), ((), ()))
_NT = (((1,), (1,)), ((), ()))
_TN = (((0,), (0,)), ((), ()))

_GELU_C = math.sqrt(2.0 / math.pi)
_GELU_A = 0.044715

RSEG, RROWS = 4, 32
WSEG, WROWS = 4, 128
PIECES = ((16, 1024), (32, 512), (64, 256), (32, 512))


def _mm(a, b, dims):
    return lax.dot_general(a.astype(BF16), b, dims, preferred_element_type=F32)


def _ln_fwd(x):
    xc = x - jnp.mean(x, axis=-1, keepdims=True)
    rstd = 1.0 / jnp.sqrt(jnp.mean(xc * xc, axis=-1, keepdims=True) + LN_EPS)
    return xc * rstd, rstd


def _ln_bwd(dh, h, rstd):
    return rstd * (dh - jnp.mean(dh, axis=-1, keepdims=True)
                   - h * jnp.mean(dh * h, axis=-1, keepdims=True))


def _gelu_fwd(a):
    t = jnp.tanh(_GELU_C * (a + _GELU_A * a * a * a))
    g = 0.5 * a * (1.0 + t)
    dg = 0.5 * (1.0 + t) + 0.5 * a * (1.0 - t * t) * (_GELU_C * (1.0 + 3.0 * _GELU_A * a * a))
    return g, dg


def _pad_rows(x):
    return jnp.concatenate([x, jnp.zeros((ROWS - x.shape[0], x.shape[1]), x.dtype)], axis=0)


def _loop(lo, hi, fn):
    if hi > lo:
        lax.fori_loop(lo, hi, lambda j, c: (fn(j), c)[1], 0)


def _num_pieces(ref, piece):
    assert ref.shape[0] % piece[0] == 0 and ref.shape[1] % piece[1] == 0
    return (ref.shape[0] // piece[0]) * (ref.shape[1] // piece[1])


def _copy_piece(src, dst, sem, piece, i, priority):
    rows, cols = piece
    nc = src.shape[1] // cols
    sl = (pl.ds(pl.multiple_of((i // nc) * rows, rows), rows),
          pl.ds(pl.multiple_of((i % nc) * cols, cols), cols))
    pltpu.make_async_copy(src.at[sl], dst.at[sl], sem).start(priority=priority)


def _interleave_weights(lo, hi, main, srcs, dsts, sems):
    for a in (0, 2):
        n = _num_pieces(srcs[a], PIECES[a])
        assert n == _num_pieces(srcs[a + 1], PIECES[a + 1])
        m = min(n, hi - lo)

        def pieces(i, a=a):
            for q in range(2):
                _copy_piece(srcs[a + q], dsts[a + q], sems[a + q], PIECES[a + q], i, q)

        _loop(0, m, lambda i, lo=lo: (main(lo + i), pieces(i)))
        _loop(m, n, pieces)
        lo += m
    _loop(lo, hi, main)


def _kernel(
    x_hbm, k_hbm, v_hbm, wq_hbm, wo_hbm, w1_hbm, b1_hbm, w2_hbm, b2_hbm, g_hbm,
    out_hbm, dx_hbm, dk_hbm, dv_hbm, dwq_hbm, dwo_hbm, dw1_hbm, db1_hbm, dw2_hbm, db2_hbm,
    kb, vb, wq, wo, w1, w2, x_s, g_s, b1_s, b2_s,
    dwq, dwo, dw1, dw2, out_s, dx_s, db1_s, db2_s,
    zero, q_t, o_t, do_t, dq_t, p_all, flat,
    ha_st, dq_st, oa_st, dxa_st, hb_st, da_st, gb_st, dxb_st,
    rsem, wsem,
):
    B, HKV, SK, DH = k_hbm.shape
    W = kb.shape[1]
    NG = B * HKV
    REP = HQ // HKV
    ZR = SK - W
    scale = DH ** -0.5

    def strip(j, seg, rows, extent):
        per = extent // rows
        grp = j // per
        return grp // (HKV // seg), (grp % (HKV // seg)) * seg, (j % per) * rows

    def window_views(j, seg, rows):
        b, h, r = strip(j, seg, rows, W)
        return ((b, pl.ds(h, seg), pl.ds(pl.multiple_of(ZR + r, rows), rows)),
                (pl.ds(b * HKV + h, seg), pl.ds(pl.multiple_of(r, rows), rows)))

    def kv_read(j):
        far, near = window_views(j, RSEG, RROWS)
        for i, (src, dst) in enumerate(((k_hbm, kb), (v_hbm, vb))):
            pltpu.make_async_copy(src.at[far], dst.at[near], rsem.at[i]).start(priority=i)

    n_read = (NG // RSEG) * (W // RROWS)
    head_start = min(16, n_read)
    _loop(0, head_start, kv_read)
    for i, (src, dst) in enumerate(((x_hbm, x_s), (g_hbm, g_s), (b1_hbm, b1_s), (b2_hbm, b2_s))):
        pltpu.make_async_copy(src, dst, rsem.at[6 + i]).start()
    for ref in (zero, q_t, do_t, flat, ha_st, dq_st, oa_st, dxa_st, hb_st, da_st, gb_st, dxb_st):
        ref[...] = jnp.zeros(ref.shape, ref.dtype)
    _interleave_weights(head_start, n_read, kv_read, (wq_hbm, wo_hbm, w1_hbm, w2_hbm),
                        (wq, wo, w1, w2), [rsem.at[2 + i] for i in range(4)])

    def zero_write(j):
        b, h, r = strip(j, WSEG, WROWS, ZR)
        for i, dst in enumerate((dk_hbm, dv_hbm)):
            pltpu.make_async_copy(
                zero, dst.at[b, pl.ds(h, WSEG), pl.ds(pl.multiple_of(r, WROWS), WROWS)],
                wsem.at[i]).start(priority=i)

    n_zero = (NG // WSEG) * (ZR // WROWS)
    n_feed = max(0, n_zero - _num_pieces(wq, PIECES[0]) - _num_pieces(w1, PIECES[2]))
    issued = [0]

    def feed(n):
        base = issued[0]
        issued[0] = min(base + n, n_feed)
        _loop(base, issued[0], zero_write)

    def head_loop(body, per_head):
        base = issued[0]
        per_head = min(per_head, (n_feed - base) // NG)
        issued[0] = base + per_head * NG

        def step(g):
            _loop(0, per_head, lambda u: zero_write(base + g * per_head + u))
            body(g)
        _loop(0, NG, step)

    feed(40)
    for i, buf in enumerate((kb, vb, wq, wo, w1, w2, x_s, g_s, b1_s, b2_s)):
        pltpu.make_async_copy(buf, buf, rsem.at[i]).wait()

    def to_tiles(val, tiles, layer):
        for b in range(B):
            for hq in range(HQ):
                row = layer * REP + hq % REP
                tiles[b * HKV + hq // REP, row:row + 1, :] = val[b:b + 1, hq * DH:(hq + 1) * DH]

    def from_tiles(tiles, layer):
        for b in range(B):
            for hq in range(HQ):
                row = layer * REP + hq % REP
                flat[b:b + 1, hq * DH:(hq + 1) * DH] = tiles[b * HKV + hq // REP, row:row + 1, :]
        return flat[...]

    def stack(ref, val, layer):
        ref[layer * B:(layer + 1) * B, :] = val[0:B, :]

    def attn_fwd(x, layer):
        h, rstd = _ln_fwd(x)
        stack(ha_st, h, layer)
        to_tiles(_mm(h, wq[...], _NN), q_t, layer)

        def body(g):
            s = _mm(q_t[g], kb[g], _NT) * scale
            e = jnp.exp(s - jnp.max(s, axis=-1, keepdims=True))
            p = e / jnp.sum(e, axis=-1, keepdims=True)
            if layer == 1:
                p_all[g] = p
            o_t[g] = _mm(p, vb[g], _NN)
        head_loop(body, 8)
        o = from_tiles(o_t, layer)
        stack(oa_st, o, layer)
        feed(8)
        return x + _mm(o, wo[...], _NN), (h, rstd)

    b1 = b1_s[...].astype(F32).reshape(1, -1)
    b2 = b2_s[...].astype(F32).reshape(1, -1)

    def mlp_fwd(x, layer):
        h, rstd = _ln_fwd(x)
        stack(hb_st, h, layer)
        g, dgelu = _gelu_fwd(_mm(h, w1[...], _NN) + b1)
        stack(gb_st, g, layer)
        feed(8)
        return x + _mm(g, w2[...], _NN) + b2, (h, rstd, dgelu)

    x0 = _pad_rows(x_s[...].astype(F32))
    x1, res_a0 = attn_fwd(x0, 0)
    x2, res_b0 = mlp_fwd(x1, 0)
    x3, res_a1 = attn_fwd(x2, 1)
    x4, res_b1 = mlp_fwd(x3, 1)
    out_s[...] = x4[0:B].astype(BF16)
    pltpu.make_async_copy(out_s, out_hbm, wsem.at[6]).start()

    def mlp_bwd(dy, res, layer):
        h, rstd, dgelu = res
        stack(dxb_st, dy, layer)
        da = _mm(dy, w2[...], _NT) * dgelu
        stack(da_st, da, layer)
        feed(8)
        return dy + _ln_bwd(_mm(da, w1[...], _NT), h, rstd)

    def attn_bwd(dy, res, layer):
        h, rstd = res
        to_tiles(_mm(dy, wo[...], _NT), do_t, layer)

        def body(g):
            p = p_all[g]
            do = do_t[g]
            dp = _mm(do, vb[g], _NT)
            ds = p * (dp - jnp.sum(p * dp, axis=-1, keepdims=True)) * scale
            dq_t[g] = _mm(ds, kb[g], _NN)
            if layer == 0:
                kb[g] = _mm(ds, q_t[g].astype(BF16), _TN).astype(BF16)
                vb[g] = _mm(p, do.astype(BF16), _TN).astype(BF16)
        head_loop(body, 8 if layer else 12)
        dq = from_tiles(dq_t, layer)
        stack(dq_st, dq, layer)
        feed(8)
        return dy + _ln_bwd(_mm(dq, wq[...], _NT), h, rstd)

    def wgrad(dst, lhs_st, rhs_st, rows):
        rhs = rhs_st[...].astype(BF16)
        for r in range(0, dst.shape[0], rows):
            dst[r:r + rows, :] = _mm(lhs_st[:, r:r + rows], rhs, _TN).astype(BF16)
        feed(8)

    d4 = _pad_rows(g_s[...].astype(F32))
    d3 = mlp_bwd(d4, res_b1, 1)
    stack(dxa_st, d3, 1)
    d2 = attn_bwd(d3, res_a1, 1)
    d1 = mlp_bwd(d2, res_b0, 0)
    stack(dxa_st, d1, 0)
    db1_s[...] = jnp.sum(da_st[...], axis=0).astype(BF16)
    db2_s[...] = jnp.sum(dxb_st[...], axis=0).astype(BF16)
    pltpu.make_async_copy(db1_s, db1_hbm, wsem.at[7]).start()
    pltpu.make_async_copy(db2_s, db2_hbm, wsem.at[8]).start()
    wgrad(dw2, gb_st, dxb_st, 256)
    wgrad(dw1, hb_st, da_st, 128)
    wgrad(dwo, oa_st, dxa_st, 512)
    d0 = attn_bwd(d1, res_a0, 0)
    dx_s[...] = d0[0:B].astype(BF16)
    pltpu.make_async_copy(dx_s, dx_hbm, wsem.at[9]).start()
    wgrad(dwq, ha_st, dq_st, 128)

    def kv_write(j):
        far, near = window_views(j, WSEG, WROWS)
        for i, (src, dst) in enumerate(((kb, dk_hbm), (vb, dv_hbm))):
            pltpu.make_async_copy(src.at[near], dst.at[far], wsem.at[i]).start(priority=i)

    feed(n_zero)
    _interleave_weights(n_feed, n_zero, zero_write, (dwq, dwo, dw1, dw2),
                        (dwq_hbm, dwo_hbm, dw1_hbm, dw2_hbm), [wsem.at[2 + i] for i in range(4)])
    _loop(0, (NG // WSEG) * (W // WROWS), kv_write)
    for i, buf in enumerate((dk_hbm, dv_hbm, dwq_hbm, dwo_hbm, dw1_hbm, dw2_hbm,
                             out_hbm, db1_hbm, db2_hbm, dx_hbm)):
        pltpu.make_async_copy(buf, buf, wsem.at[i]).wait()


@jax.jit
def pallas_interleave_layers__sliding_block_cached__dense_activation_gelu__decode_kernel(
    A_x: jax.Array,
    A_k_cache: jax.Array,
    A_v_cache: jax.Array,
    A_wq: jax.Array,
    A_wo: jax.Array,
    B_x: jax.Array,
    B_w1: jax.Array,
    B_b1: jax.Array,
    B_w2: jax.Array,
    B_b2: jax.Array,
    grad_out: jax.Array,
):
    del B_x
    B, SQ, D = A_x.shape
    _, HKV, SK, DH = A_k_cache.shape
    FF = B_w1.shape[1]
    W = min(4096, max(256, SK // 4))
    NG = B * HKV
    assert SQ == 1 and 2 * B <= ROWS and 2 * (HQ // HKV) == ROWS
    assert HKV % RSEG == 0 and HKV % WSEG == 0
    assert W % RROWS == 0 and W % WROWS == 0 and SK % RROWS == 0 and SK % WROWS == 0

    def like(a):
        return jax.ShapeDtypeStruct(a.shape, a.dtype)

    def vmem(shape, dtype=BF16):
        return pltpu.VMEM(tuple(shape), dtype)

    act = jax.ShapeDtypeStruct((B, D), A_x.dtype)
    hbm = pl.BlockSpec(memory_space=pltpu.HBM)
    weights = [vmem(w.shape) for w in (A_wq, A_wo, B_w1, B_w2)]
    small = [vmem((B, D)), vmem((B, D)), vmem((FF,)), vmem((D,))]
    tile = vmem((NG, ROWS, DH), F32)
    res = pl.pallas_call(
        _kernel,
        out_shape=(act, act, like(A_k_cache), like(A_v_cache), like(A_wq), like(A_wo),
                   like(B_w1), like(B_b1), like(B_w2), like(B_b2)),
        in_specs=[hbm] * 10,
        out_specs=(hbm,) * 10,
        scratch_shapes=[
            vmem((NG, W, DH)), vmem((NG, W, DH)), *weights, *small,
            *weights, *small,
            vmem((WSEG, WROWS, DH)), tile, tile, tile, tile,
            vmem((NG, ROWS, W), F32), vmem((ROWS, HQ * DH), F32),
            vmem((ROWS, D), F32), vmem((ROWS, HQ * DH), F32),
            vmem((ROWS, HQ * DH), F32), vmem((ROWS, D), F32),
            vmem((ROWS, D), F32), vmem((ROWS, FF), F32),
            vmem((ROWS, FF), F32), vmem((ROWS, D), F32),
            pltpu.SemaphoreType.DMA((10,)), pltpu.SemaphoreType.DMA((10,)),
        ],
        compiler_params=pltpu.CompilerParams(vmem_limit_bytes=100 * 2**20),
    )(A_x.reshape(B, D), A_k_cache, A_v_cache, A_wq, A_wo, B_w1, B_b1, B_w2, B_b2,
      grad_out.reshape(B, D))
    return (res[0].reshape(B, SQ, D), res[1].reshape(B, SQ, D), *res[2:])
```
